```python
import os as _os
_os.environ.setdefault("JAX_PLATFORMS", "cpu")
import jax
import jax.numpy as jnp

def _softmax(x, axis=-1):
    return jax.nn.softmax(x, axis=axis)
def _gelu(x):
    return jax.nn.gelu(x, approximate=True)
def _silu(x):
    return jax.nn.silu(x)
def _sigmoid(x):
    return jax.nn.sigmoid(x)
def _layernorm(x, axis=-1, eps=1e-5):
    m = jnp.mean(x, axis=axis, keepdims=True)
    v = jnp.var(x, axis=axis, keepdims=True)
    return (x - m) / jnp.sqrt(v + eps)
def _scatter_add(tgt, idx, src, axis=0):
    return tgt.at[idx].add(src)
def _segment_sum(src, seg, n):
    return jax.ops.segment_sum(src, seg, n)
class _Rng:
    def __init__(self, key):
        self._k = key
    def _next(self):
        self._k, sub = jax.random.split(self._k)
        return sub
    def normal(self, shape):
        return jax.random.normal(self._next(), shape, dtype=jnp.bfloat16)
    def randint(self, lo, hi, shape):
        return jax.random.randint(self._next(), shape, lo, hi, dtype=jnp.int32)
    def uniform(self, shape, lo=0.0, hi=1.0):
        return jax.random.uniform(self._next(), shape, jnp.bfloat16, lo, hi)
    def permutation(self, n):
        return jax.random.permutation(self._next(), n)


kernel_name = 'sequential_preLN__mha_block__swiglu_ffn__prompt'

def setup_inputs():
    _rng = _Rng(jax.random.key(int.from_bytes(__import__("os").urandom(4), "little")))
    _w = (lambda a: (lambda t: t.astype(jnp.bfloat16) if jnp.issubdtype(t.dtype, jnp.floating) else t)(jnp.asarray(a)))
    def _A_setup():
        B, S, D, H = 1, 2048, 640, 32
        return {
            "x": _w((lambda *s: _rng.normal(s) * 0.05)(B, S, D)),
            "wqkv": _w((lambda *s: _rng.normal(s) * 0.05)(D, 3 * D)),
            "wo": _w((lambda *s: _rng.normal(s) * 0.05)(D, D)),
        }
    _A_in = _A_setup()

    def _B_setup():
        B, S, D, F = 1, 2048, 640, 1728
        return {
            "x": _w((lambda *s: _rng.normal(s) * 0.05)(B, S, D)),
            "w_gate": _w((lambda *s: _rng.normal(s) * 0.05)(D, F)),
            "w_up": _w((lambda *s: _rng.normal(s) * 0.05)(D, F)),
            "w_down": _w((lambda *s: _rng.normal(s) * 0.05)(F, D)),
        }
    _B_in = _B_setup()

    return {
        "A_x": _A_in["x"],
        "A_wqkv": _A_in["wqkv"],
        "A_wo": _A_in["wo"],
        "B_x": _B_in["x"],
        "B_w_gate": _B_in["w_gate"],
        "B_w_up": _B_in["w_up"],
        "B_w_down": _B_in["w_down"],
    }

def reference(A_x, A_wqkv, A_wo, B_x, B_w_gate, B_w_up, B_w_down):
    def _A_ref(x, wqkv, wo):
        B, S, D = x.shape
        H = 32
        Dh = D // H
        qkv = (lambda x, *d: x.transpose(*d))((x @ wqkv).reshape(B, S, 3, H, Dh), 2, 0, 3, 1, 4)
        q, k, v = qkv[0], qkv[1], qkv[2]
        scores = jnp.einsum("bhqd,bhkd->bhqk", q, k) * (Dh ** -0.5)
        p = _softmax(scores, axis=-1)
        o = jnp.einsum("bhqk,bhkd->bhqd", p, v)
        return (lambda x, *d: x.transpose(*d))(o, 0, 2, 1, 3).reshape(B, S, D) @ wo

    def _B_ref(x, w_gate, w_up, w_down):
        g = _silu(x @ w_gate)
        u = x @ w_up
        return (g * u) @ w_down

    x = A_x
    h = x + _A_ref(_layernorm(x, axis=-1), A_wqkv, A_wo)
    h2 = h + _B_ref(_layernorm(h, axis=-1), B_w_gate, B_w_up, B_w_down)
    return h2
```

```python
import functools
import math


import jax
import jax.numpy as jnp
from jax import lax
import jax.experimental.pallas as pl
import jax.experimental.pallas.tpu as pltpu

S = 2048
D = 640
H = 32
DH = 20
F = 1728
EPS = 1e-5
LANES = 128
NT = D // LANES
NX = 4
VR = 24
TA = 512
TQ = 512
TK = 128
TM = 256
NB = 4
DIST = 2
UNROLL = 8
FM = (F // LANES) * LANES
FL = F - FM
FC = 1664
QSCALE = (DH ** -0.5) * math.log2(math.e)

_NN_DIMS = (((1,), (0,)), ((), ()))
_NT_DIMS = (((1,), (1,)), ((), ()))


def _ln(x):
    m = jnp.mean(x, axis=-1, keepdims=True)
    xc = x - m
    v = jnp.mean(xc * xc, axis=-1, keepdims=True)
    return xc * lax.rsqrt(v + EPS)


def _silu_mul(g, u):
    return g * jax.nn.sigmoid(g) * u


def _kernel(x_hbm, wqkv_hbm, wo_hbm, wgt_hbm, wut_hbm, wd_hbm, o_hbm,
            x_ref, wqkv_ref, wo_ref, wgu_ref, wd_ref, out_ref,
            q_ref, k_ref, vt_ref, wvt_ref, ot_ref, h_ref, hn_ref,
            s0_ref, s1_ref, s2_ref, s3_ref, m0_ref, m1_ref, m2_ref, m3_ref,
            in_sems, out_sems):
    f32 = jnp.float32
    bf16 = jnp.bfloat16
    s_refs = (s0_ref, s1_ref, s2_ref, s3_ref)
    m_refs = (m0_ref, m1_ref, m2_ref, m3_ref)
    NA = S // TA

    x_cp = [pltpu.make_async_copy(x_hbm.at[pl.ds(c * TA, TA), :], x_ref.at[pl.ds(c * TA, TA), :],
                                  in_sems.at[c]) for c in range(NA)]
    wqk_cp = pltpu.make_async_copy(wqkv_hbm.at[:, pl.ds(0, 2 * D)], wqkv_ref.at[:, pl.ds(0, 2 * D)],
                                   in_sems.at[NA])
    wv_cp = pltpu.make_async_copy(wqkv_hbm.at[:, pl.ds(2 * D, D)], wqkv_ref.at[:, pl.ds(2 * D, D)],
                                  in_sems.at[NA + 1])
    late_cp = [
        pltpu.make_async_copy(wo_hbm, wo_ref, in_sems.at[NA + 2]),
        pltpu.make_async_copy(wgt_hbm.at[pl.ds(0, FM), :], wgu_ref.at[pl.ds(0, FM), :], in_sems.at[NA + 3]),
        pltpu.make_async_copy(wut_hbm.at[pl.ds(0, FM), :], wgu_ref.at[pl.ds(FM, FM), :], in_sems.at[NA + 4]),
        pltpu.make_async_copy(wgt_hbm.at[pl.ds(FM, FL), :], wgu_ref.at[pl.ds(2 * FM, FL), :], in_sems.at[NA + 5]),
        pltpu.make_async_copy(wut_hbm.at[pl.ds(FM, FL), :], wgu_ref.at[pl.ds(2 * FM + FL, FL), :], in_sems.at[NA + 6]),
        pltpu.make_async_copy(wd_hbm, wd_ref, in_sems.at[NA + 7]),
    ]
    x_cp[0].start()
    wqk_cp.start()
    wv_cp.start()
    for c in range(1, NA):
        x_cp[c].start()

    row4 = lax.broadcasted_iota(jnp.int32, (VR - DH, TA), 0)
    tail = jnp.where(row4 == 0, 1.0, 0.0).astype(f32)
    lane_a = lax.broadcasted_iota(jnp.int32, (TA, LANES), 1)

    def ln1(r0):
        return _ln(x_ref[pl.ds(r0, TA), :].astype(f32)).astype(bf16)

    def proj_qk(r0, xn):
        qk = jnp.dot(xn, wqkv_ref[:, 0:2 * D], preferred_element_type=f32)
        for dst, base, scale in ((q_ref, 0, QSCALE), (k_ref, D, None)):
            tiles = []
            for t in range(NT):
                v = qk[:, base + t * LANES: base + (t + 1) * LANES]
                if scale is not None:
                    v = v * scale
                tiles.append(v)
                dst[t, pl.ds(r0, TA), :] = v.astype(bf16)
            for t in range(NX):
                dst[NT + t, pl.ds(r0, TA), :] = jnp.where(
                    lane_a >= 64, tiles[t], tiles[t + 1]).astype(bf16)

    def proj_v(r0, xn):
        vt = lax.dot_general(wvt_ref[...], xn, _NT_DIMS, preferred_element_type=f32)
        for h in range(H):
            vt_ref[h, :, pl.ds(r0, TA)] = jnp.concatenate(
                [vt[h * DH:(h + 1) * DH, :], tail], axis=0)

    x_cp[0].wait()
    xn0 = ln1(0)
    wqk_cp.wait()
    proj_qk(0, xn0)
    wv_cp.wait()
    wvt_ref[...] = wqkv_ref[:, 2 * D:3 * D].astype(f32).T.astype(bf16)
    proj_v(0, xn0)
    for c in range(1, NA):
        x_cp[c].wait()
    for cp in late_cp:
        cp.start()

    def phase_a(c, carry):
        r0 = pl.multiple_of(c * TA, TA)
        xn = ln1(r0)
        proj_qk(r0, xn)
        proj_v(r0, xn)
        return carry

    lax.fori_loop(1, NA, phase_a, 0)

    NQ = S // TQ
    NI = NQ * H
    NK = S // TK
    lane_q = lax.broadcasted_iota(jnp.int32, (TQ, LANES), 1)

    def step(iq, bq, ip, bp):
        if iq is not None:
            h = iq % H
            q0 = pl.multiple_of((iq // H) * TQ, TQ)
            off = (h * DH) % LANES
            g = (h * DH) // LANES
            t = jnp.where(off > LANES - DH, g + NT, g)
            qt = q_ref[t, pl.ds(q0, TQ), :]
            rel = (lane_q - off) & (LANES - 1)
            qm = jnp.where(rel < DH, qt, jnp.zeros_like(qt))
            m = None
        if ip is not None:
            hp = ip % H
            mp = m_refs[bp][0:1, :]
            acc = None
        for kc in range(NK):
            sl = slice(kc * TK, (kc + 1) * TK)
            if iq is not None:
                s = lax.dot_general(k_ref[t, sl, :], qm, _NT_DIMS, preferred_element_type=f32)
                s_refs[bq][sl, :] = s
                mc = jnp.max(s.reshape(TK // 8, 8, TQ), axis=0)
                m = mc if m is None else jnp.maximum(m, mc)
            if ip is not None:
                p = jnp.exp2(s_refs[bp][sl, :] - mp).astype(bf16)
                d = lax.dot_general(vt_ref[hp, :, sl], p, _NN_DIMS, preferred_element_type=f32)
                acc = d if acc is None else acc + d
        if iq is not None:
            m_refs[bq][...] = jnp.broadcast_to(jnp.max(m, axis=0, keepdims=True), (8, TQ))
        if ip is not None:
            return acc[0:DH, :] / acc[DH:DH + 1, :]
        return None

    def store_pair(i_even, oa, ob):
        q0 = pl.multiple_of((i_even // H) * TQ, TQ)
        r0 = pl.multiple_of((i_even % H) * DH, 2 * DH)
        ot_ref[pl.ds(r0, 2 * DH), pl.ds(q0, TQ)] = jnp.concatenate([oa, ob], axis=0)

    def steps(p0, n):
        outs = []
        for u in range(n):
            ip = p0 + u
            iq = ip + DIST
            if isinstance(iq, int) and iq >= NI:
                iq = None
            outs.append(step(iq, (u + DIST) % NB, ip, u % NB))
            if u % 2 == 1:
                store_pair(ip - 1, outs[-2], outs[-1])

    for i in range(DIST):
        step(i, i % NB, None, None)

    NLOOP = NI // UNROLL - 1

    def attn_body(j, carry):
        steps(j * UNROLL, UNROLL)
        return carry

    lax.fori_loop(0, NLOOP, attn_body, 0)
    for cp in late_cp:
        cp.wait()
    steps(NLOOP * UNROLL, UNROLL)

    for c in range(S // TM):
        r0 = c * TM
        o = ot_ref[:, pl.ds(r0, TM)].T.astype(bf16)
        hres = x_ref[pl.ds(r0, TM), :].astype(f32) + jnp.dot(
            o, wo_ref[...], preferred_element_type=f32)
        h_ref[pl.ds(r0, TM), :] = hres
        hn_ref[pl.ds(r0, TM), :] = _ln(hres).astype(bf16)

    def out_cp(c):
        r0 = pl.multiple_of(c * TM, TM)
        return pltpu.make_async_copy(out_ref.at[pl.ds(r0, TM), :], o_hbm.at[pl.ds(r0, TM), :],
                                     out_sems.at[c])

    def phase_c(c, carry):
        r0 = pl.multiple_of(c * TM, TM)
        hn = hn_ref[pl.ds(r0, TM), :]
        y = h_ref[pl.ds(r0, TM), :]
        gul = lax.dot_general(hn, wgu_ref[2 * FM:2 * FM + 2 * FL, :], _NT_DIMS,
                              preferred_element_type=f32)
        al = _silu_mul(gul, pltpu.roll(gul, FL, 1))[:, 0:FL].astype(bf16)
        y = y + jnp.dot(al, wd_ref[FM:F, :], preferred_element_type=f32)
        for f0 in range(0, FM, FC):
            fc = min(FC, FM - f0)
            g = lax.dot_general(hn, wgu_ref[f0:f0 + fc, :], _NT_DIMS, preferred_element_type=f32)
            u = lax.dot_general(hn, wgu_ref[FM + f0:FM + f0 + fc, :], _NT_DIMS,
                                preferred_element_type=f32)
            a = _silu_mul(g, u).astype(bf16)
            y = y + jnp.dot(a, wd_ref[f0:f0 + fc, :], preferred_element_type=f32)
        out_ref[pl.ds(r0, TM), :] = y.astype(out_ref.dtype)
        out_cp(c).start()
        return carry

    lax.fori_loop(0, S // TM, phase_c, 0)
    for c in range(S // TM):
        out_cp(c).wait()


@jax.jit
def pallas_sequential_preLN__mha_block__swiglu_ffn__prompt_kernel(
    A_x, A_wqkv, A_wo, B_x, B_w_gate, B_w_up, B_w_down,
):
    del B_x
    bf16 = jnp.bfloat16
    f32 = jnp.float32
    x = A_x.reshape(S, D)
    out = pl.pallas_call(
        _kernel,
        out_shape=jax.ShapeDtypeStruct((S, D), A_x.dtype),
        in_specs=[pl.BlockSpec(memory_space=pl.ANY)] * 6,
        out_specs=pl.BlockSpec(memory_space=pl.ANY),
        scratch_shapes=[
            pltpu.VMEM((S, D), bf16),
            pltpu.VMEM((D, 3 * D), bf16),
            pltpu.VMEM((D, D), bf16),
            pltpu.VMEM((2 * F, D), bf16),
            pltpu.VMEM((F, D), bf16),
            pltpu.VMEM((S, D), bf16),
            pltpu.VMEM((NT + NX, S, LANES), bf16),
            pltpu.VMEM((NT + NX, S, LANES), bf16),
            pltpu.VMEM((H, VR, S), f32),
            pltpu.VMEM((D, D), bf16),
            pltpu.VMEM((D, S), f32),
            pltpu.VMEM((S, D), f32),
            pltpu.VMEM((S, D), bf16),
        ] + [pltpu.VMEM((S, TQ), f32)] * NB + [pltpu.VMEM((8, TQ), f32)] * NB + [
            pltpu.SemaphoreType.DMA((S // TA + 8,)),
            pltpu.SemaphoreType.DMA((S // TM,)),
        ],
        compiler_params=pltpu.CompilerParams(vmem_limit_bytes=110 * 1024 * 1024),
    )(x, A_wqkv, A_wo, B_w_gate.T, B_w_up.T, B_w_down)
    return out.reshape(1, S, D)
```

```python
import functools
import math

import jax
import jax.numpy as jnp
from jax import lax
import jax.experimental.pallas as pl
import jax.experimental.pallas.tpu as pltpu

S = 2048
D = 640
H = 32
DH = 20
F = 1728
EPS = 1e-5
LANES = 128
NT = D // LANES
VR = 24
TA = 512
TKB = 128
TQ = 512
TK = 128
TM = 256
NB = 4
DIST = 2
UNROLL = 8
FM = (F // LANES) * LANES
FL = F - FM
QSCALE = (DH ** -0.5) * math.log2(math.e)

_NN_DIMS = (((1,), (0,)), ((), ()))
_NT_DIMS = (((1,), (1,)), ((), ()))


def _ln(x):
    m = jnp.mean(x, axis=-1, keepdims=True)
    xc = x - m
    v = jnp.mean(xc * xc, axis=-1, keepdims=True)
    return xc * lax.rsqrt(v + EPS)


def _silu_mul(g, u):
    return g * jax.nn.sigmoid(g) * u


def _kernel(x_hbm, wqkv_hbm, wo_hbm, wgt_hbm, wut_hbm, wd_hbm, o_hbm,
            x_ref, wqkv_ref, wo_ref, wgu_ref, wd_ref, out_ref,
            xn_ref, k_ref, qt_ref, vt_ref, wqvt_ref, ot_ref, h_ref, hn_ref,
            s0_ref, s1_ref, s2_ref, s3_ref, m0_ref, m1_ref, m2_ref, m3_ref,
            in_sems, out_sems):
    f32 = jnp.float32
    bf16 = jnp.bfloat16
    s_refs = (s0_ref, s1_ref, s2_ref, s3_ref)
    m_refs = (m0_ref, m1_ref, m2_ref, m3_ref)
    NA = S // TA

    XP = ((0, 256), (256, 768), (1024, 1024))
    x_cp = [pltpu.make_async_copy(x_hbm.at[pl.ds(r0, n), :], x_ref.at[pl.ds(r0, n), :],
                                  in_sems.at[c]) for c, (r0, n) in enumerate(XP)]
    w_cp = [pltpu.make_async_copy(wqkv_hbm.at[:, pl.ds(j * D, D)], wqkv_ref.at[:, pl.ds(j * D, D)],
                                  in_sems.at[NA + j]) for j in range(3)]
    late_cp = [
        pltpu.make_async_copy(wo_hbm, wo_ref, in_sems.at[NA + 3]),
        pltpu.make_async_copy(wgt_hbm.at[pl.ds(0, FM), :], wgu_ref.at[pl.ds(0, FM), :], in_sems.at[NA + 4]),
        pltpu.make_async_copy(wut_hbm.at[pl.ds(0, FM), :], wgu_ref.at[pl.ds(FM, FM), :], in_sems.at[NA + 5]),
        pltpu.make_async_copy(wgt_hbm.at[pl.ds(FM, FL), :], wgu_ref.at[pl.ds(2 * FM, FL), :], in_sems.at[NA + 6]),
        pltpu.make_async_copy(wut_hbm.at[pl.ds(FM, FL), :], wgu_ref.at[pl.ds(2 * FM + FL, FL), :], in_sems.at[NA + 7]),
        pltpu.make_async_copy(wd_hbm, wd_ref, in_sems.at[NA + 8]),
    ]
    x_cp[0].start()
    w_cp[1].start()

    row4 = lax.broadcasted_iota(jnp.int32, (VR - DH, TA), 0)
    tail = jnp.where(row4 == 0, 1.0, 0.0).astype(f32)
    lane_a = lax.broadcasted_iota(jnp.int32, (TKB, LANES), 1)

    def ln1(r0, n):
        rows = pl.ds(r0, n)
        xn_ref[rows, :] = _ln(x_ref[rows, :].astype(f32)).astype(bf16)

    def proj_k(r0, n):
        for r in range(n // TKB):
            rows = pl.ds(r0 + r * TKB, TKB)
            k = jnp.dot(xn_ref[rows, :], wqkv_ref[:, D:2 * D], preferred_element_type=f32)
            tiles = [k[:, t * LANES:(t + 1) * LANES] for t in range(NT)]
            for h in range(H):
                g, off = divmod(h * DH, LANES)
                src = tiles[g]
                if off + DH > LANES:
                    src = jnp.where(lane_a >= LANES // 2, src, tiles[g + 1])
                if off:
                    src = pltpu.roll(src, LANES - off, 1)
                k_ref[h, rows, :] = src.astype(bf16)

    def proj_qv(c):
        cols = pl.ds(c * TA, TA)
        qv = lax.dot_general(wqvt_ref[...], xn_ref[cols, :], _NT_DIMS, preferred_element_type=f32)
        for h in range(H):
            qt_ref[h, 0:DH, cols] = qv[h * DH:(h + 1) * DH, :] * QSCALE
            vt_ref[h, :, cols] = jnp.concatenate(
                [qv[D + h * DH:D + (h + 1) * DH, :], tail], axis=0)

    x_cp[0].wait()
    ln1(0, 256)
    x_cp[1].start()
    w_cp[1].wait()
    proj_k(0, 256)
    w_cp[0].start()
    w_cp[2].start()
    x_cp[1].wait()
    ln1(256, 256)
    proj_k(256, 256)
    ln1(512, 256)
    proj_k(512, 256)
    ln1(768, 256)
    x_cp[2].start()
    w_cp[0].wait()
    w_cp[2].wait()
    proj_k(768, 256)
    wqvt_ref[0:D, :] = wqkv_ref[:, 0:D].astype(f32).T.astype(bf16)
    wqvt_ref[D:2 * D, :] = wqkv_ref[:, 2 * D:3 * D].astype(f32).T.astype(bf16)
    proj_qv(0)
    for cp in late_cp:
        cp.start()
    x_cp[2].wait()
    proj_qv(1)
    ln1(1024, 512)
    ln1(1536, 512)
    proj_k(1024, 512)
    proj_qv(2)
    proj_k(1536, 512)
    proj_qv(3)

    NQ = S // TQ
    NI = NQ * H
    NK = S // TK

    def step(iq, bq, ip, bp, fillers=None):
        if iq is not None:
            h = iq % H
            q0 = pl.multiple_of((iq // H) * TQ, TQ)
            qm = qt_ref[h, 0:DH, pl.ds(q0, TQ)]
            m = None
        if ip is not None:
            hp = ip % H
            mp = m_refs[bp][0:1, :]
            acc = None
        for kc in range(NK):
            sl = slice(kc * TK, (kc + 1) * TK)
            if iq is not None:
                s = lax.dot_general(k_ref[h, sl, 0:DH], qm, _NN_DIMS, preferred_element_type=f32)
                s_refs[bq][sl, :] = s
                mc = jnp.max(s.reshape(TK // 8, 8, TQ), axis=0)
                m = mc if m is None else jnp.maximum(m, mc)
            if ip is not None:
                p = jnp.exp2(s_refs[bp][sl, :] - mp).astype(bf16)
                d = lax.dot_general(vt_ref[hp, :, sl], p, _NN_DIMS, preferred_element_type=f32)
                acc = d if acc is None else acc + d
            if fillers and kc in fillers:
                fillers[kc]()
        if iq is not None:
            m_refs[bq][...] = jnp.broadcast_to(jnp.max(m, axis=0, keepdims=True), (8, TQ))
        if ip is not None:
            return acc[0:DH, :] / acc[DH:DH + 1, :]
        return None

    def store_pair(i_even, oa, ob):
        q0 = pl.multiple_of((i_even // H) * TQ, TQ)
        r0 = pl.multiple_of((i_even % H) * DH, 2 * DH)
        ot_ref[pl.ds(r0, 2 * DH), pl.ds(q0, TQ)] = jnp.concatenate([oa, ob], axis=0)

    def steps(p0, n, fillers=None):
        outs = []
        for u in range(n):
            ip = p0 + u
            iq = ip + DIST
            if isinstance(iq, int) and iq >= NI:
                iq = None
            outs.append(step(iq, (u + DIST) % NB, ip, u % NB, fillers.get(u) if fillers else None))
            if u % 2 == 1:
                store_pair(ip - 1, outs[-2], outs[-1])

    for i in range(DIST):
        step(i, i % NB, None, None)

    NLOOP = NI // UNROLL - 1

    def attn_body(j, carry):
        steps(j * UNROLL, UNROLL)
        return carry

    lax.fori_loop(0, NLOOP, attn_body, 0)
    for cp in late_cp:
        cp.wait()

    def c1_t(c):
        rows = pl.ds(c * TM, TM)
        xn_ref[rows, :] = ot_ref[:, rows].T.astype(bf16)

    def c1_mm(c, n):
        rows = pl.ds(c * TM, TM)
        cols = pl.ds(n * LANES, LANES)
        h_ref[rows, cols] = x_ref[rows, cols].astype(f32) + jnp.dot(
            xn_ref[rows, :], wo_ref[:, cols], preferred_element_type=f32)

    def c1_ln(c):
        rows = pl.ds(c * TM, TM)
        hn_ref[rows, :] = _ln(h_ref[rows, :]).astype(bf16)

    def c1_full(c):
        rows = pl.ds(c * TM, TM)
        o = ot_ref[:, rows].T.astype(bf16)
        hres = x_ref[rows, :].astype(f32) + jnp.dot(o, wo_ref[...], preferred_element_type=f32)
        h_ref[rows, :] = hres
        hn_ref[rows, :] = _ln(hres).astype(bf16)

    P = functools.partial
    fillers = {UNROLL - DIST - 1: {4: P(c1_t, 0), 10: P(c1_t, 1)}}
    for j in range(DIST):
        fillers[UNROLL - DIST + j] = {1 + 3 * n: P(c1_mm, j, n) for n in range(NT)}
    steps(NLOOP * UNROLL, UNROLL, fillers)
    for c in range(DIST, S // TM):
        c1_full(c)
        if c - DIST < DIST:
            c1_ln(c - DIST)

    def out_cp(c):
        r0 = pl.multiple_of(c * TM, TM)
        return pltpu.make_async_copy(out_ref.at[pl.ds(r0, TM), :], o_hbm.at[pl.ds(r0, TM), :],
                                     out_sems.at[c])

    def phase_c(c, carry):
        r0 = pl.multiple_of(c * TM, TM)
        hn = hn_ref[pl.ds(r0, TM), :]
        y = h_ref[pl.ds(r0, TM), :]
        gul = lax.dot_general(hn, wgu_ref[2 * FM:2 * FM + 2 * FL, :], _NT_DIMS,
                              preferred_element_type=f32)
        al = _silu_mul(gul, pltpu.roll(gul, FL, 1))[:, 0:FL].astype(bf16)
        y = y + jnp.dot(al, wd_ref[FM:F, :], preferred_element_type=f32)
        g = lax.dot_general(hn, wgu_ref[0:FM, :], _NT_DIMS, preferred_element_type=f32)
        u = lax.dot_general(hn, wgu_ref[FM:2 * FM, :], _NT_DIMS, preferred_element_type=f32)
        a = _silu_mul(g, u).astype(bf16)
        y = y + jnp.dot(a, wd_ref[0:FM, :], preferred_element_type=f32)
        out_ref[pl.ds(r0, TM), :] = y.astype(out_ref.dtype)
        out_cp(c).start()
        return carry

    lax.fori_loop(0, S // TM, phase_c, 0)
    for c in range(S // TM):
        out_cp(c).wait()


@jax.jit
def pallas_sequential_preLN__mha_block__swiglu_ffn__prompt_kernel(
    A_x, A_wqkv, A_wo, B_x, B_w_gate, B_w_up, B_w_down,
):
    del B_x
    bf16 = jnp.bfloat16
    f32 = jnp.float32
    x = A_x.reshape(S, D)
    out = pl.pallas_call(
        _kernel,
        out_shape=jax.ShapeDtypeStruct((S, D), A_x.dtype),
        in_specs=[pl.BlockSpec(memory_space=pl.ANY)] * 6,
        out_specs=pl.BlockSpec(memory_space=pl.ANY),
        scratch_shapes=[
            pltpu.VMEM((S, D), bf16),
            pltpu.VMEM((D, 3 * D), bf16),
            pltpu.VMEM((D, D), bf16),
            pltpu.VMEM((2 * F, D), bf16),
            pltpu.VMEM((F, D), bf16),
            pltpu.VMEM((S, D), bf16),
            pltpu.VMEM((S, D), bf16),
            pltpu.VMEM((H, S, LANES), bf16),
            pltpu.VMEM((H, VR, S), f32),
            pltpu.VMEM((H, VR, S), f32),
            pltpu.VMEM((2 * D, D), bf16),
            pltpu.VMEM((D, S), f32),
            pltpu.VMEM((S, D), f32),
            pltpu.VMEM((S, D), bf16),
        ] + [pltpu.VMEM((S, TQ), f32)] * NB + [pltpu.VMEM((8, TQ), f32)] * NB + [
            pltpu.SemaphoreType.DMA((S // TA + 9,)),
            pltpu.SemaphoreType.DMA((S // TM,)),
        ],
        compiler_params=pltpu.CompilerParams(vmem_limit_bytes=120 * 1024 * 1024),
    )(x, A_wqkv, A_wo, B_w_gate.T, B_w_up.T, B_w_down)
    return out.reshape(1, S, D)
```

```python
import functools
import math

import jax
import jax.numpy as jnp
from jax import lax
import jax.experimental.pallas as pl
import jax.experimental.pallas.tpu as pltpu

S = 2048
D = 640
H = 32
DH = 20
F = 1728
EPS = 1e-5
LANES = 128
NT = D // LANES
VR = 24
TA = 512
TKB = 128
TQ = 512
TK = 128
TM = 256
NB = 4
DIST = 2
UNROLL = 12
TAILN = 8
FM = (F // LANES) * LANES
FL = F - FM
QSCALE = (DH ** -0.5) * math.log2(math.e)
X_PIECES = ((0, 256), (256, 768), (1024, 1024))
N_IN_SEMS = 13

_NN_DIMS = (((1,), (0,)), ((), ()))
_NT_DIMS = (((1,), (1,)), ((), ()))


def _ln(x):
    m = jnp.mean(x, axis=-1, keepdims=True)
    xc = x - m
    v = jnp.mean(xc * xc, axis=-1, keepdims=True)
    return xc * lax.rsqrt(v + EPS)


def _silu_mul(g, u):
    return g * jax.nn.sigmoid(g) * u


def _kernel(x_hbm, wqkv_hbm, wo_hbm, wgt_hbm, wut_hbm, wd_hbm, o_hbm,
            x_ref, wqkv_ref, wo_ref, wgu_ref, wd_ref, out_ref,
            xn_ref, k_ref, qt_ref, vt_ref, wqvt_ref, ot_ref, h_ref, hn_ref,
            *rest):
    f32 = jnp.float32
    bf16 = jnp.bfloat16
    s_refs = rest[:NB]
    m_refs = rest[NB:2 * NB]
    in_sems, out_sems = rest[2 * NB:]

    x_cp = [pltpu.make_async_copy(x_hbm.at[pl.ds(r0, n), :], x_ref.at[pl.ds(r0, n), :],
                                  in_sems.at[c]) for c, (r0, n) in enumerate(X_PIECES)]
    w_cp = [pltpu.make_async_copy(wqkv_hbm.at[:, pl.ds(j * D, D)], wqkv_ref.at[:, pl.ds(j * D, D)],
                                  in_sems.at[4 + j]) for j in range(3)]
    late_cp = [
        pltpu.make_async_copy(wo_hbm, wo_ref, in_sems.at[7]),
        pltpu.make_async_copy(wgt_hbm.at[pl.ds(0, FM), :], wgu_ref.at[pl.ds(0, FM), :],
                              in_sems.at[8]),
        pltpu.make_async_copy(wut_hbm.at[pl.ds(0, FM), :], wgu_ref.at[pl.ds(FM, FM), :],
                              in_sems.at[9]),
        pltpu.make_async_copy(wgt_hbm.at[pl.ds(FM, FL), :], wgu_ref.at[pl.ds(2 * FM, FL), :],
                              in_sems.at[10]),
        pltpu.make_async_copy(wut_hbm.at[pl.ds(FM, FL), :], wgu_ref.at[pl.ds(2 * FM + FL, FL), :],
                              in_sems.at[11]),
        pltpu.make_async_copy(wd_hbm, wd_ref, in_sems.at[12]),
    ]
    x_cp[0].start()
    w_cp[1].start()
    x_cp[1].start()
    w_cp[0].start()
    w_cp[2].start()
    x_cp[2].start()
    for cp in late_cp:
        cp.start()

    row4 = lax.broadcasted_iota(jnp.int32, (VR - DH, TA), 0)
    tail = jnp.where(row4 == 0, 1.0, 0.0).astype(f32)
    lane_a = lax.broadcasted_iota(jnp.int32, (TKB, LANES), 1)

    def ln1(r0, n):
        rows = pl.ds(r0, n)
        xn_ref[rows, :] = _ln(x_ref[rows, :].astype(f32)).astype(bf16)

    def proj_k(r0, n):
        for r in range(n // TKB):
            rows = pl.ds(r0 + r * TKB, TKB)
            k = jnp.dot(xn_ref[rows, :], wqkv_ref[:, D:2 * D], preferred_element_type=f32)
            tiles = [k[:, t * LANES:(t + 1) * LANES] for t in range(NT)]
            for h in range(H):
                g, off = divmod(h * DH, LANES)
                src = tiles[g]
                if off + DH > LANES:
                    src = jnp.where(lane_a >= LANES // 2, src, tiles[g + 1])
                if off:
                    src = pltpu.roll(src, LANES - off, 1)
                k_ref[h, rows, :] = src.astype(bf16)

    def proj_qv(c):
        cols = pl.ds(c * TA, TA)
        qv = lax.dot_general(wqvt_ref[...], xn_ref[cols, :], _NT_DIMS, preferred_element_type=f32)
        for h in range(H):
            qt_ref[h, 0:DH, cols] = qv[h * DH:(h + 1) * DH, :] * QSCALE
            v = qv[D + h * DH:D + (h + 1) * DH, :]
            vt_ref[h, :, cols] = jnp.concatenate([v, tail] if h % 2 == 0 else [tail, v], axis=0)

    x_cp[0].wait()
    ln1(0, 256)
    w_cp[1].wait()
    proj_k(0, 256)
    x_cp[1].wait()
    ln1(256, 256)
    proj_k(256, 256)
    ln1(512, 256)
    proj_k(512, 256)
    ln1(768, 256)
    w_cp[0].wait()
    w_cp[2].wait()
    proj_k(768, 256)
    wqvt_ref[0:D, :] = wqkv_ref[:, 0:D].astype(f32).T.astype(bf16)
    wqvt_ref[D:2 * D, :] = wqkv_ref[:, 2 * D:3 * D].astype(f32).T.astype(bf16)
    proj_qv(0)
    x_cp[2].wait()
    proj_qv(1)
    ln1(1024, 512)
    ln1(1536, 512)
    proj_k(1024, 512)
    proj_qv(2)
    proj_k(1536, 512)
    proj_qv(3)

    NQ = S // TQ
    NI = NQ * H
    NK = S // TK

    def step(iq, bq, ip, bp, odd, fillers=None):
        if iq is not None:
            h = iq % H
            q0 = pl.multiple_of((iq // H) * TQ, TQ)
            qm = qt_ref[h, 0:DH, pl.ds(q0, TQ)]
            m = None
        if ip is not None:
            hp = ip % H
            mp = m_refs[bp][0:1, :]
            acc = None
        for kc in range(NK):
            sl = slice(kc * TK, (kc + 1) * TK)
            if iq is not None:
                s = lax.dot_general(k_ref[h, sl, 0:DH], qm, _NN_DIMS, preferred_element_type=f32)
                s_refs[bq][sl, :] = s
                mc = jnp.max(s.reshape(TK // 8, 8, TQ), axis=0)
                m = mc if m is None else jnp.maximum(m, mc)
            if ip is not None:
                p = jnp.exp2(s_refs[bp][sl, :] - mp).astype(bf16)
                d = lax.dot_general(vt_ref[hp, :, sl], p, _NN_DIMS, preferred_element_type=f32)
                acc = d if acc is None else acc + d
            if fillers and kc in fillers:
                fillers[kc]()
        if iq is not None:
            m_refs[bq][...] = jnp.broadcast_to(jnp.max(m, axis=0, keepdims=True), (8, TQ))
        if ip is not None:
            l = acc[0:1, :] if odd else acc[DH:DH + 1, :]
            r = pl.reciprocal(l, approx=True)
            r = r * (2.0 - l * r)
            o = acc * r
            return o[VR - DH:VR, :] if odd else o[0:DH, :]
        return None

    def store_pair(i_even, oa, ob):
        q0 = pl.multiple_of((i_even // H) * TQ, TQ)
        r0 = pl.multiple_of((i_even % H) * DH, 2 * DH)
        ot_ref[pl.ds(r0, 2 * DH), pl.ds(q0, TQ)] = jnp.concatenate([oa, ob], axis=0)

    def steps(p0, n, fillers=None):
        outs = []
        for u in range(n):
            ip = p0 + u
            iq = ip + DIST
            if isinstance(iq, int) and iq >= NI:
                iq = None
            outs.append(step(iq, (u + DIST) % NB, ip, u % NB, u % 2 == 1,
                             fillers.get(u) if fillers else None))
            if u % 2 == 1:
                store_pair(ip - 1, outs[-2], outs[-1])

    for i in range(DIST):
        step(i, i % NB, None, None, False)

    NLOOP = (NI - TAILN) // UNROLL

    def attn_body(j, carry):
        steps(j * UNROLL, UNROLL)
        return carry

    lax.fori_loop(0, NLOOP, attn_body, 0)
    for cp in late_cp:
        cp.wait()

    def c1_t(c):
        rows = pl.ds(c * TM, TM)
        xn_ref[rows, :] = ot_ref[:, rows].T.astype(bf16)

    def c1_mm(c, n):
        rows = pl.ds(c * TM, TM)
        cols = pl.ds(n * LANES, LANES)
        h_ref[rows, cols] = x_ref[rows, cols].astype(f32) + jnp.dot(
            xn_ref[rows, :], wo_ref[:, cols], preferred_element_type=f32)

    def c1_ln(c):
        rows = pl.ds(c * TM, TM)
        hn_ref[rows, :] = _ln(h_ref[rows, :]).astype(bf16)

    def c1_full(r0, n):
        rows = pl.ds(r0, n)
        o = ot_ref[:, rows].T.astype(bf16)
        hres = x_ref[rows, :].astype(f32) + jnp.dot(o, wo_ref[...], preferred_element_type=f32)
        h_ref[rows, :] = hres
        hn_ref[rows, :] = _ln(hres).astype(bf16)

    P = functools.partial
    fillers = {TAILN - DIST - 1: {2 + 4 * j: P(c1_t, j) for j in range(DIST)}}
    for j in range(DIST):
        fillers[TAILN - DIST + j] = {1 + 3 * n: P(c1_mm, j, n) for n in range(NT)}
    steps(NLOOP * UNROLL, TAILN, fillers)
    for c in range(2 * DIST, 2 * S // TM):
        c1_full(c * TM // 2, TM // 2)
        if c - 2 * DIST < 2 * DIST and c % 2 == 1:
            c1_ln((c - 2 * DIST) // 2)

    def out_cp(c):
        r0 = pl.multiple_of(c * TM, TM)
        return pltpu.make_async_copy(out_ref.at[pl.ds(r0, TM), :], o_hbm.at[pl.ds(r0, TM), :],
                                     out_sems.at[c])

    def phase_c(c, carry):
        r0 = pl.multiple_of(c * TM, TM)
        hn = hn_ref[pl.ds(r0, TM), :]
        y = h_ref[pl.ds(r0, TM), :]
        gul = lax.dot_general(hn, wgu_ref[2 * FM:2 * FM + 2 * FL, :], _NT_DIMS,
                              preferred_element_type=f32)
        al = _silu_mul(gul, pltpu.roll(gul, FL, 1))[:, 0:FL].astype(bf16)
        y = y + jnp.dot(al, wd_ref[FM:F, :], preferred_element_type=f32)
        g = lax.dot_general(hn, wgu_ref[0:FM, :], _NT_DIMS, preferred_element_type=f32)
        u = lax.dot_general(hn, wgu_ref[FM:2 * FM, :], _NT_DIMS, preferred_element_type=f32)
        a = _silu_mul(g, u).astype(bf16)
        y = y + jnp.dot(a, wd_ref[0:FM, :], preferred_element_type=f32)
        out_ref[pl.ds(r0, TM), :] = y.astype(out_ref.dtype)
        out_cp(c).start()
        return carry

    lax.fori_loop(0, S // TM, phase_c, 0)
    for c in range(S // TM):
        out_cp(c).wait()


@jax.jit
def pallas_sequential_preLN__mha_block__swiglu_ffn__prompt_kernel(
    A_x: jax.Array,
    A_wqkv: jax.Array,
    A_wo: jax.Array,
    B_x: jax.Array,
    B_w_gate: jax.Array,
    B_w_up: jax.Array,
    B_w_down: jax.Array,
):
    del B_x
    bf16 = jnp.bfloat16
    f32 = jnp.float32
    x = A_x.reshape(S, D)
    out = pl.pallas_call(
        _kernel,
        out_shape=jax.ShapeDtypeStruct((S, D), A_x.dtype),
        in_specs=[pl.BlockSpec(memory_space=pl.ANY)] * 6,
        out_specs=pl.BlockSpec(memory_space=pl.ANY),
        scratch_shapes=[
            pltpu.VMEM((S, D), bf16),
            pltpu.VMEM((D, 3 * D), bf16),
            pltpu.VMEM((D, D), bf16),
            pltpu.VMEM((2 * F, D), bf16),
            pltpu.VMEM((F, D), bf16),
            pltpu.VMEM((S, D), bf16),
            pltpu.VMEM((S, D), bf16),
            pltpu.VMEM((H, S, LANES), bf16),
            pltpu.VMEM((H, VR, S), f32),
            pltpu.VMEM((H, VR, S), f32),
            pltpu.VMEM((2 * D, D), bf16),
            pltpu.VMEM((D, S), f32),
            pltpu.VMEM((S, D), f32),
            pltpu.VMEM((S, D), bf16),
        ] + [pltpu.VMEM((S, TQ), f32)] * NB + [pltpu.VMEM((8, TQ), f32)] * NB + [
            pltpu.SemaphoreType.DMA((N_IN_SEMS,)),
            pltpu.SemaphoreType.DMA((S // TM,)),
        ],
        compiler_params=pltpu.CompilerParams(vmem_limit_bytes=120 * 1024 * 1024),
    )(x, A_wqkv, A_wo, B_w_gate.T, B_w_up.T, B_w_down)
    return out.reshape(1, S, D)
```
